```python
import os as _os
_os.environ.setdefault("JAX_PLATFORMS", "cpu")
import jax
import jax.numpy as jnp

def _softmax(x, axis=-1):
    return jax.nn.softmax(x, axis=axis)
def _gelu(x):
    return jax.nn.gelu(x, approximate=True)
def _silu(x):
    return jax.nn.silu(x)
def _sigmoid(x):
    return jax.nn.sigmoid(x)
def _layernorm(x, axis=-1, eps=1e-5):
    m = jnp.mean(x, axis=axis, keepdims=True)
    v = jnp.var(x, axis=axis, keepdims=True)
    return (x - m) / jnp.sqrt(v + eps)
def _scatter_add(tgt, idx, src, axis=0):
    return tgt.at[idx].add(src)
def _segment_sum(src, seg, n):
    return jax.ops.segment_sum(src, seg, n)
class _Rng:
    def __init__(self, key):
        self._k = key
    def _next(self):
        self._k, sub = jax.random.split(self._k)
        return sub
    def normal(self, shape):
        return jax.random.normal(self._next(), shape, dtype=jnp.bfloat16)
    def randint(self, lo, hi, shape):
        return jax.random.randint(self._next(), shape, lo, hi, dtype=jnp.int32)
    def uniform(self, shape, lo=0.0, hi=1.0):
        return jax.random.uniform(self._next(), shape, jnp.bfloat16, lo, hi)
    def permutation(self, n):
        return jax.random.permutation(self._next(), n)


kernel_name = 'interleave_layers__sliding_local_dilated__mixer_s_mlp__prompt'

def setup_inputs():
    _rng = _Rng(jax.random.key(int.from_bytes(__import__("os").urandom(4), "little")))
    _w = (lambda a: (lambda t: t.astype(jnp.bfloat16) if jnp.issubdtype(t.dtype, jnp.floating) else t)(jnp.asarray(a)))
    def _A_setup():
        B, S, D = 1, 2048, 448
        return {
            "x": _w((lambda *s: _rng.normal(s) * 0.05)(B, S, D)),
            "wqkv": _w((lambda *s: _rng.normal(s) * 0.05)(D, 3 * D)),
            "wo": _w((lambda *s: _rng.normal(s) * 0.05)(D, D)),
        }
    _A_in = _A_setup()

    def _B_setup():
        B, S, D, F = 1, 2048, 448, 1792
        return {
            "x":  _w((lambda *s: _rng.normal(s) * 0.05)(B, S, D)),
            "w1": _w((lambda *s: _rng.normal(s) * 0.8)(D, D) * (D ** -0.5)),
            "w2": _w((lambda *s: _rng.normal(s) * 0.8)(D, D) * (D ** -0.5)),
            "w3": _w((lambda *s: _rng.normal(s) * 0.8)(D, F) * (D ** -0.5)),
            "w4": _w((lambda *s: _rng.normal(s) * 0.8)(F, D) * (F ** -0.5)),
        }
    _B_in = _B_setup()

    return {
        "A_x": _A_in["x"],
        "A_wqkv": _A_in["wqkv"],
        "A_wo": _A_in["wo"],
        "B_x": _B_in["x"],
        "B_w1": _B_in["w1"],
        "B_w2": _B_in["w2"],
        "B_w3": _B_in["w3"],
        "B_w4": _B_in["w4"],
    }

def reference(A_x, A_wqkv, A_wo, B_x, B_w1, B_w2, B_w3, B_w4):
    def _A_ref(x, wqkv, wo):
        B, S, D = x.shape
        H = 16; Dh = D // H
        W, dil = 8, 2
        qkv = (lambda x, *d: x.transpose(*d))((x @ wqkv).reshape(B, S, 3, H, Dh), 2, 0, 3, 1, 4)
        q, k, v = qkv[0], qkv[1], qkv[2]
        scale = Dh ** -0.5
        pos = jnp.arange(S)
        off = jnp.arange(W) * dil
        idx = pos[:, None] - off[None, :]
        mask = idx >= 0
        idx_c = jnp.where(mask, idx, 0).reshape(-1)
        kg = k[:, :, idx_c, :].reshape(B, H, S, W, Dh)
        vg = v[:, :, idx_c, :].reshape(B, H, S, W, Dh)
        logits = jnp.einsum("bhsd,bhswd->bhsw", q, kg) * scale
        logits = jnp.where(mask[None, None, :, :], logits, -1e9)
        attn = _softmax(logits, axis=-1)
        o = jnp.einsum("bhsw,bhswd->bhsd", attn, vg)
        return (lambda x, *d: x.transpose(*d))(o, 0, 2, 1, 3).reshape(B, S, D) @ wo

    def _B_ref(x, w1, w2, w3, w4):
        B, S, D = x.shape
        h = _gelu(_layernorm(x, axis=-1) @ w1)
        c = D // 4
        g0 = jnp.pad(h[:, :, 0*c:1*c], ((0, 0), (1, 0), (0, 0)))[:, :S, :]
        g1 = jnp.pad(h[:, :, 1*c:2*c], ((0, 0), (0, 1), (0, 0)))[:, 1:, :]
        g2 = jnp.pad(h[:, :, 2*c:3*c], ((0, 0), (2, 0), (0, 0)))[:, :S, :]
        g3 = jnp.pad(h[:, :, 3*c:   ], ((0, 0), (0, 2), (0, 0)))[:, 2:, :]
        hs = jnp.concatenate([g0, g1, g2, g3], axis=-1) @ w2
        x1 = x + hs
        h2 = _gelu(_layernorm(x1, axis=-1) @ w3) @ w4
        return x1 + h2

    x = A_x
    x = x + _A_ref(_layernorm(x, axis=-1), A_wqkv, A_wo)
    x = x + _B_ref(_layernorm(x, axis=-1), B_w1, B_w2, B_w3, B_w4)
    x = x + _A_ref(_layernorm(x, axis=-1), A_wqkv, A_wo)
    x = x + _B_ref(_layernorm(x, axis=-1), B_w1, B_w2, B_w3, B_w4)
    return x
```

```python
import functools
import math

import jax
import jax.numpy as jnp
from jax import lax
import jax.experimental.pallas as pl
import jax.experimental.pallas.tpu as pltpu

FILL = (dict(spread=0.75, delay=1, qk_piece=1, pv_piece=2, tcost=55, nbuf=5), (
    ("Pq", 0, 8), ("Pk", 0, -13), ("Pv", 0, 26), ("Pwo", 0, 71), ("Pw1", 0, 134), ("Pw2", 0, 146),
    ("Pw3", 0, 163), ("Pw4", 0, 198), ("ldx", 0, -5), ("ldx", 1, 23), ("ldx", 2, 9), ("ldx", 3, 65),
    ("ldx", 4, 79), ("ldx", 5, 100), ("ldx", 6, 135), ("ldx", 7, 142), ("ln1", 0, -4), ("ln1", 1, 24),
    ("ln1", 2, 10), ("ln1", 3, 66), ("budget", 0, 300), ("q", 0, 28), ("k", 0, 35), ("probs", 0, 49),
    ("q", 2, 42), ("v", 0, 35), ("ln1", 4, 80), ("attn", 0, 48), ("v", 1, 56), ("q", 1, 63), ("budget", 0, 300),
    ("k", 1, 70), ("ln1", 5, 101), ("probs", 1, 112), ("v", 2, 77), ("k", 2, 84), ("ln1", 6, 136),
    ("wo", 0, 99), ("attn", 1, 111), ("probs", 2, 189), ("q", 3, 98), ("v", 3, 105), ("budget", 0, 300),
    ("q", 4, 112), ("k", 3, 119), ("ln1", 7, 143), ("v", 4, 126), ("q", 5, 133), ("k", 5, 140), ("w1", 0, 168),
    ("budget", 0, 330), ("wo", 1, 162), ("attn", 2, 188), ("k", 4, 161), ("v", 6, 168), ("v", 7, 175),
    ("v", 5, 175), ("q", 7, 175), ("budget", 0, 360), ("k", 7, 175), ("q", 6, 175), ("w1", 1, 168),
    ("shift", 0, 224), ("k", 6, 175), ("w2", 0, 35), ("ln4", 0, 163)))
EARLY = (dict(spread=0.65, delay=2, qk_piece=4, pv_piece=4, nbuf=5), (
    ("budget", 0, 210), ("out", 4, 30), ("probs", 0, 70), ("attn", 0, 100), ("wo", 1, 15), ("w30", 3, 40),
    ("w31", 3, 46), ("w1", 1, 36), ("shift", 2, 58), ("budget", 0, 236), ("w32", 3, 70), ("w40", 3, 0),
    ("w33", 3, 62), ("w2", 2, 0), ("ln4", 2, 77), ("budget", 0, 224), ("w41", 3, 0), ("w42", 3, 0),
    ("w43", 3, 0)))
STEADY = (dict(spread=0.8, delay=3, qk_piece=2, pv_piece=4, nbuf=3), (
    ("budget", 0, 188), ("ln1", 0, 7), ("out", 4, 30), ("ln4", 3, 29), ("wo", 1, 22), ("k", 0, 24),
    ("q", 0, -6), ("probs", 0, 85), ("v", 0, 45), ("attn", 0, 125), ("budget", 0, 190), ("w1", 1, 48),
    ("shift", 2, 83), ("w30", 3, 67), ("w31", 3, 69), ("w32", 3, 79), ("w40", 3, 0), ("w33", 3, 59),
    ("budget", 0, 187), ("w41", 3, 0), ("w42", 3, 0), ("w2", 2, 0), ("w43", 3, 0)))
DRAIN = (dict(spread=0.85, delay=1, qk_piece=2, pv_piece=2, tcost=55, nbuf=5), (
    ("ln4", 13, 5), ("out", 12, -15), ("budget", 0, 190), ("wo", 15, 50), ("w30", 13, 15), ("w1", 15, 47),
    ("shift", 14, 40), ("w31", 13, 36), ("w32", 13, 9), ("w40", 13, 0), ("budget", 0, 150), ("w2", 14, 30),
    ("shift", 15, 70), ("w41", 13, 0), ("w33", 13, 31), ("ln4", 14, 35), ("w42", 13, 0), ("w43", 13, 0),
    ("out", 13, 15), ("w30", 14, 45), ("budget", 0, 110), ("w31", 14, 66), ("w32", 14, 39), ("w2", 15, 60),
    ("w40", 14, 30), ("w33", 14, 61), ("ln4", 15, 65), ("w41", 14, 30), ("budget", 0, 160), ("w42", 14, 30),
    ("w43", 14, 30), ("out", 14, 45), ("w30", 15, 75), ("w31", 15, 96), ("send", 14, 30), ("w32", 15, 69),
    ("w33", 15, 91), ("budget", 0, 120), ("w40", 15, 60), ("w41", 15, 60), ("w42", 15, 60), ("w43", 15, 60),
    ("out", 15, 75), ("send", 15, 60)))
W3_CHUNKS = (256, 256, 128, 256)
W4_CHUNKS = (0, 512, 0, 384)

S, D, F = 2048, 448, 1792
H, DH, W, DIL = 16, 28, 8, 2
TS = 256
NL = TS // 128
NS = S // TS
K1 = 256
K2 = D - K1
HN = D // 2
NBUF = 5
X_SPANS = {"x0": (0, 1), "x1": (1, 4), "x2": (4, NS)}
SYNC = {15: (("v", "x1"), ("w1", "w2", "x2")), 49: (("wo", "w1", "w2", "x2"), ("w3", "w4")), 105: (("w3", "w4"), ())}
ARRIVAL = {key: at for at, (keys, _) in SYNC.items() for key in keys}
AFTER = {"q": ("v", "x1"), "k": ("wo",)}
QKV_COLS = (0, 512, 896, 3 * D)
EPS = 1e-5
f32, bf16, u32 = jnp.float32, jnp.bfloat16, jnp.uint32
GC0 = math.sqrt(2.0 / math.pi)
GS = (GC0 * 0.044715) ** (1.0 / 3.0)


def _cat(xs, axis):
    return jnp.concatenate(xs, axis=axis)


def _pack(x):
    return pltpu.pack_elementwise([x[0:8], x[8:16]], packed_dtype=bf16)


def _halves(x):
    return _cat([pltpu.unpack_elementwise(x, index=i, packed_dtype=bf16, unpacked_dtype=f32) for i in range(2)], 0)


def _unpack(x):
    return pltpu.bitcast(x, bf16)


def _mean(p):
    while p.shape[0] > 8:
        p = p[:p.shape[0] // 2] + p[p.shape[0] // 2:]
    return jnp.sum(p, axis=0, keepdims=True) * (1.0 / D)


def _gelu_scaled(y):
    return y * jnp.tanh(y * (y * y + GC0 / GS)) + y


def _act_operands(b11, b12, b21, b22):
    return (b11 + b22, b11, b12 - b22, b21 - b11, b22, b11 + b12, b21 + b22)


def _weight_operands(a11, a12, a21, a22):
    return (a11 + a22, a21 + a22, a11, a22, a11 + a12, a21 - a11, a12 - a22)


def _kernel(x_hbm, wqkv_hbm, wo_hbm, w1_hbm, w2_hbm, w3_hbm, w4_hbm, o_hbm,
            xin, wqkv_v, wo_v, w1_v, w2_v, w3_v, w4_v, tmp, tmp2,
            wqkv_s, wo_s, w1_s, w2_s, w3_s, w4_s,
            xa, xb, xn_s, x1_s, h_s, q_s, k_s, v_s, p_s, of_s, st_s,
            a1, o_s, a2, g_s, a3, b4, acc0, acc1, prod0, prod1, prod2, prod3, prod4, prod_w2, sink, ost, zero_s, sem_in, sem_w, sem_out):
    lane = lax.broadcasted_iota(jnp.int32, (1, 128), 1)

    def out_copy(c):
        return pltpu.make_async_copy(ost.at[c], o_hbm.at[:, pl.ds(c * TS, TS)], sem_out.at[c])

    w_copies = {}
    for i, name in enumerate("qkv"):
        span = pl.ds(QKV_COLS[i], QKV_COLS[i + 1] - QKV_COLS[i])
        w_copies[name] = pltpu.make_async_copy(wqkv_hbm.at[:, span], wqkv_v.at[0:D, span], sem_w.at[i])
    for i, (name, src, dst) in enumerate((("wo", wo_hbm, wo_v), ("w1", w1_hbm, w1_v), ("w2", w2_hbm, w2_v),
                                          ("w3", w3_hbm, w3_v), ("w4", w4_hbm, w4_v))):
        w_copies[name] = pltpu.make_async_copy(src, dst.at[0:D], sem_w.at[3 + i])

    for i, (name, (c0, c1)) in enumerate(X_SPANS.items()):
        span = pl.ds(c0 * TS, (c1 - c0) * TS)
        w_copies[name] = pltpu.make_async_copy(x_hbm.at[:, span], xin.at[:, span], sem_in.at[i])
    started, landed, sent = [], [], []

    def start(key):
        if key not in started:
            started.append(key)
            w_copies[key].start()

    def fetch(key):
        if key not in landed:
            start(key)
            landed.append(key)
            w_copies[key].wait()
            for nxt in AFTER.get(key, ()):
                start(nxt)

    def x_key(c):
        return next(name for name, (c0, c1) in X_SPANS.items() if c0 <= c < c1)

    def transposed(blk):
        kk, nn = blk.shape
        if nn < 128:
            blk = _cat([blk, jnp.zeros((kk, 128 - nn), bf16)], 1)
        if kk < 128:
            blk = _cat([blk, jnp.zeros((128 - kk, 128), bf16)], 0)
        return pltpu.bitcast(blk.T, u32)

    def transpose_to_tmp(src, n_lo, n_hi):
        for n0 in range(n_lo, n_hi, 128):
            nn = min(128, n_hi - n0)
            for j in range(4):
                tmp[j, n0 // 2:n0 // 2 + 64, :] = transposed(src[j * 128:min(D, j * 128 + 128), n0:n0 + nn])
                yield tune["tcost"], [tmp], (src if j < 3 or n0 + 128 < n_hi else tmp)

    def store_operands(dst, j, r0, a11, a12, a21, a22):
        for p, t in enumerate(_weight_operands(a11, a12, a21, a22)):
            dst[p, j, r0 // 2:r0 // 2 + 8, :] = _pack(t)

    def prep_plain(name, src, dst, n):
        fetch(name)
        yield from transpose_to_tmp(src, 0, n)
        yield from split_plain(dst, n)

    def parity_split(j, r):
        a, b = [_halves(tmp[j, pl.ds(r // 2 + i, 8, stride=2), :]) for i in range(2)]
        return [_cat([a[i:i + 8], b[i:i + 8]], 0) for i in (0, 8)]

    def split_plain(dst, n):
        for r in range(0, n // 2, 32):
            for j in range(2):
                blocks = [parity_split(jj, rr) for rr in (r, n // 2 + r) for jj in (j, j + 2)]
                for i in range(2):
                    store_operands(dst, j, r + 16 * i, *[t[i] for t in blocks])
                yield 60, [dst], tmp

    def by_head(ref, j, first):
        lo = _halves(ref[j, pl.ds(first, 8, stride=DH // 2), :])
        hi = _halves(ref[j, pl.ds(first + 8 * (DH // 2), 8, stride=DH // 2), :])
        return [_cat([lo[i:i + 8], hi[i:i + 8]], 0) for i in (0, 8)]

    def prep_qkv(part):
        fetch("qkv"[part])
        yield from transpose_to_tmp(wqkv_v, QKV_COLS[part], QKV_COLS[part + 1])
        for e in range(DH // 4):
            top, bot = part * HN + e, part * HN + e + DH // 4
            for j in range(2):
                blocks = [by_head(tmp, jj, r) for r in (top, bot) for jj in (j, j + 2)]
                for i in range(2):
                    store_operands(wqkv_s, j, part * HN + (2 * e + i) * H, *[t[i] for t in blocks])
                yield 60, [wqkv_s], tmp

    def prep_wo():
        fetch("wo")
        for j in range(4):
            blk = wo_v[0:D, j * 128:min(D, j * 128 + 128)]
            if blk.shape[1] < 128:
                blk = _cat([blk, jnp.zeros((D, 128 - blk.shape[1]), bf16)], 1)
            tmp2[j, 0:HN, :] = pltpu.bitcast(blk, u32)
            yield 100, [tmp2], (wo_v if j < 3 else tmp2)
        for j in range(4):
            for kt in range(4):
                rows = [_unpack(_pack(_unpack(_pack(t)).astype(f32)))
                        for e in range(kt * 4, min(DH // 2, kt * 4 + 4)) for t in by_head(tmp2, j, e)]
                tmp[kt, j * 64:j * 64 + 64, :] = transposed(_cat(rows, 0))
                yield tune["tcost"] + 50, [tmp], (tmp2 if j < 3 or kt < 3 else tmp)
        yield from split_plain(wo_s, D)

    def prep_w4():
        fetch("w4")
        hk = F // 2
        for j in range(hk // 128):
            base = j % 2 * D
            for b in range(2):
                tmp[b, base // 2:base // 2 + HN, :] = pltpu.bitcast(
                    w4_v[0:D, b * hk + j * 128:b * hk + (j + 1) * 128], u32)
            yield 200, [tmp], tmp
            for r in range(0, HN, 32):
                blocks = [parity_split(b, base + rr) for rr in (r, HN + r) for b in range(2)]
                for i in range(2):
                    store_operands(w4_s, j, r + 16 * i, *[t[i] for t in blocks])
                yield 60, [w4_s], (tmp if r + 32 < HN else w4_v)

    def load_x(c):
        fetch(x_key(c))
        for l in range(NL):
            for r in range(0, D, 16):
                xa[c, l, r:r + 16, :] = _halves(pltpu.bitcast(xin[r:r + 16, c * TS + l * 128:c * TS + (l + 1) * 128], u32))
            yield 200, [xa], None

    preps = dict(q=(lambda: prep_qkv(0), wqkv_v), k=(lambda: prep_qkv(1), wqkv_v), v=(lambda: prep_qkv(2), wqkv_v),
                 wo=(prep_wo, wo_v), w1=(lambda: prep_plain("w1", w1_v, w1_s, D), w1_v),
                 w2=(lambda: prep_plain("w2", w2_v, w2_s, D), w2_v), w3=(lambda: prep_plain("w3", w3_v, w3_s, F), w3_v), w4=(prep_w4, w4_v))

    tasks = []
    slot, credit, zero, budget = [0], [0], [None], [0]

    def spawn(name, deadline, gen, src=None, delay=0, after=()):
        tasks.append([deadline, name, gen, src, slot[0] + delay, after])
        tasks.sort(key=lambda t: t[0])

    def advance(task, after=None):
        if after is not None and task[3] is not None:
            z, ref = zero[0], task[3]
            n = 32 // ref.dtype.itemsize
            spare = pl.ds(pl.multiple_of(ref.shape[-2] - n + z, n), n)
            ref[(z,) * (len(ref.shape) - 2) + (spare, slice(0, 128))] = pltpu.bitcast(after, ref.dtype)
        step = next(task[2], None)
        if step is None:
            tasks.remove(task)
            return 0, []
        cost, done, task[3] = step
        return cost, done

    def finish(*names):
        for task in [t for t in tasks if not names or t[1] in names]:
            if task[5]:
                finish(*task[5])
            while any(task is t for t in tasks):
                advance(task)

    def product(w, b):
        if started:
            fetch("k")
        z = zero[0]
        m = jnp.dot(_cat([_unpack(t) for t in w], 1), _unpack(b), preferred_element_type=f32)
        slot[0] += 1
        if started and slot[0] in SYNC:
            for key in SYNC[slot[0]][0]:
                fetch(key)
            for key in SYNC[slot[0]][1]:
                start(key)
        total = budget[0] * len(w) * m.shape[0] / (2 * HN)
        left = min(credit[0], 0) + total
        made = []
        while left > 0:
            task = next((t for t in tasks if t[4] <= slot[0] and not any(u[1] in t[5] for u in tasks)), None)
            if task is None:
                break
            r = 8 * int((1 - left / total) * tune["spread"] * m.shape[0] // 8)
            cost, done = advance(task, m[r:r + 8])
            left -= cost
            made.extend(d for d in done if not any(d is e for e in made))
        credit[0] = left
        made = [d if isinstance(d, jax.Array) else
                d[(z,) * (len(d.shape) - 2) + (pl.ds(pl.multiple_of(z, 8), 8), slice(None))] for d in made]
        if made:
            d = functools.reduce(jnp.bitwise_or, [pltpu.bitcast(d, u32) for d in made])
            sink[z] = jnp.tanh(pltpu.bitcast(d, f32))
        return m

    def strassen(w_ref, r0, rn, b_ref, out):
        z = zero[0]
        for p in range(7):
            out[z, p, 0:rn, :] = product([w_ref[p, j, r0 // 2:(r0 + rn) // 2, :] for j in range(2)], b_ref[p])

    def quadrants(ref, r, paired=True):
        z, e = zero[0], r - r % 32 // 2
        m1, m2, m3, m4, m5, m6, m7 = [
            _cat([ref[z, p, e:e + 8, :], ref[z, p, e + 16:e + 24, :]], 0) if paired else ref[z, p, r:r + 16, :]
            for p in range(7)]
        return (m1 + m4) + (m7 - m5), m3 + m5, m2 + m4, (m1 - m2) + (m3 + m6)

    def tiles(ref, r, paired=True):
        return zip((0, 1, 0, 1), (r, r, HN + r, HN + r), quadrants(ref, r, paired))

    def put_operands(dst, get, cost, src):
        for r in range(0, K1, 16):
            rows = slice(r // 2, r // 2 + 8)
            b11, b12 = get(0, r), get(1, r)
            if r < K2:
                for p, t in enumerate(_act_operands(b11, b12, get(0, K1 + r), get(1, K1 + r))):
                    dst[p, rows, :] = _pack(t)
                yield 17 + 8 * cost, [dst], src
            else:
                t = _pack(b11)
                dst[0, rows, :] = t
                dst[1, rows, :] = t
                dst[2, rows, :] = _pack(b12)
                dst[5, rows, :] = _pack(b11 + b12)
                yield 5 + 4 * cost, [dst], src

    def ln_stats(total, load, row, scale, src):
        for l in range(NL):
            st_s[row + 2 * l] = jnp.broadcast_to(_mean(total[l]), (8, 128))
        yield 0, [], src
        for l in range(NL):
            m = st_s[row + 2 * l, 0:1, :]
            p = None
            for r0 in range(0, D, 112):
                for r in range(r0, r0 + 112, 16):
                    xc = load(l, r) - m
                    p = xc * xc if p is None else p + xc * xc
                yield 42, [p[0:8], p[8:16]], src
            rs = lax.rsqrt(_mean(p) + EPS)
            st_s[row + 2 * l + 1] = jnp.broadcast_to(rs if scale == 1.0 else rs * scale, (8, 128))
        yield 0, [], src

    def normed(load, row):
        return lambda l, r: (load(l, r) - st_s[row + 2 * l, 0:1, :]) * st_s[row + 2 * l + 1, 0:1, :]

    def ln1_task(c):
        def load(l, r):
            return xa[c, l, r:r + 16, :]
        tot = [None] * NL
        for l in range(NL):
            tot[l] = functools.reduce(jnp.add, [load(l, r) for r in range(0, D, 16)])
            yield 56, [tot[l][0:8], tot[l][8:16]], xa
        yield from ln_stats(tot, load, 0, 1.0, xa)
        yield from put_operands(a1.at[c & 3], normed(load, 0), 2, xa)

    def q_task(c, src):
        for r0 in range(0, HN, 16):
            for l, r, y in tiles(src, r0, False):
                q_s[c * NL + l, r:r + 16, :] = y
            yield 16, [q_s], src

    def kv_task(c, src, dst):
        for r0 in range(0, HN, 16):
            for l, r, y in tiles(src, r0, False):
                dst[c * NL + l + 1, r // 2:r // 2 + 8, :] = _pack(y)
            yield 20, [dst], src

    def shifted(prev, cur, w):
        if w:
            cur = pltpu.roll(jnp.where(lane >= 128 - DIL * w, prev, cur), DIL * w, 1)
        return _halves(cur)

    def probs_task(c):
        nd = tune["qk_piece"]
        for l in range(NL):
            t = c * NL + l
            for d0 in range(0, DH, nd):
                z = zero[0]
                lg = [p_s[z + l, w] if d0 else None for w in range(W)]
                for d in range(d0, d0 + nd):
                    qv = q_s[t, d * H:(d + 1) * H, :]
                    prev, cur = k_s[t, d * 8:(d + 1) * 8, :], k_s[t + 1, d * 8:(d + 1) * 8, :]
                    for w in range(W):
                        p = qv * shifted(prev, cur, w)
                        lg[w] = p if lg[w] is None else lg[w] + p
                if d0 + nd == DH:
                    for w in range(W):
                        lg[w] = lg[w] * (DH ** -0.5)
                        if w and l == 0:
                            lg[w] = jnp.where(lane + t * 128 >= DIL * w, lg[w], -1e9)
                    m = functools.reduce(jnp.maximum, lg)
                    e = [jnp.exp(a - m) for a in lg]
                    inv = 1.0 / functools.reduce(jnp.add, e)
                    lg = [a * inv for a in e]
                for w in range(W):
                    p_s[z + l, w] = lg[w]
                yield 55 * nd + (130 if d0 + nd == DH else 0), [p_s], k_s

    def attn_out_task(c):
        nd = tune["pv_piece"]
        for l in range(NL):
            t = c * NL + l
            for d0 in range(0, DH, nd):
                z = zero[0]
                e = [p_s[z + l, w] for w in range(W)]
                for d in range(d0, d0 + nd):
                    prev, cur = v_s[t, d * 8:(d + 1) * 8, :], v_s[t + 1, d * 8:(d + 1) * 8, :]
                    if l == 0:
                        prev = jnp.where(lane + c * 128 >= 128, prev, jnp.broadcast_to(cur[:, 0:1], cur.shape))
                    pr = [e[w] * shifted(prev, cur, w) for w in range(W)]
                    of_s[l, d * H:(d + 1) * H, :] = (
                        ((pr[0] + pr[1]) + (pr[2] + pr[3])) + ((pr[4] + pr[5]) + (pr[6] + pr[7])))
                yield 55 * nd, [of_s], (v_s if (d0 + nd < DH or l < NL - 1) else of_s)
        yield from put_operands(o_s, lambda l, r: of_s[l, r:r + 16, :], 0, of_s)

    def wo_task(c, src):
        tot = [None] * NL
        for r0 in range(0, HN, 16):
            for l, r, y in tiles(src, r0):
                x = xa[c, l, r:r + 16, :] + y
                xb[c, l, r:r + 16, :] = x
                tot[l] = x if tot[l] is None else tot[l] + x
            yield 32, [xb], (src if r0 + 16 < HN else xb)
        yield from ln_stats(tot, lambda l, r: xb[c, l, r:r + 16, :], 4, 1.0, xb)
        n = normed(lambda l, r: xb[c, l, r:r + 16, :], 4)
        for l in range(NL):
            tot[l] = None
            for r0 in range(0, D, 112):
                for r in range(r0, r0 + 112, 16):
                    xn = n(l, r)
                    xn_s[c, l, r:r + 16, :] = xn
                    tot[l] = xn if tot[l] is None else tot[l] + xn
                yield 42, [xn_s], (xb if (r0 + 112 < D or l < NL - 1) else xn_s)
        yield from ln_stats(tot, lambda l, r: xn_s[c, l, r:r + 16, :], 8, GS, xn_s)
        yield from put_operands(a2, normed(lambda l, r: xn_s[c, l, r:r + 16, :], 8), 2, xn_s)

    def w1_task(c, src):
        for r0 in range(0, HN, 16):
            for l, r, y in tiles(src, r0):
                h_s[c * NL + l + 1, r:r + 16, :] = _gelu_scaled(y)
            yield 56, [h_s], src

    def shift_task(c):
        def get(l, r):
            t = c * NL + l + 1
            sh = (1, -1, 2, -2)[r // (D // 4)]
            cur = h_s[t, r:r + 16, :]
            if sh > 0:
                y = jnp.where(lane >= 128 - sh, h_s[t - 1, r:r + 16, :], cur)
            else:
                y = jnp.where(lane < -sh, h_s[t + 1, r:r + 16, :], cur)
            return pltpu.roll(y, sh % 128, 1)
        yield from put_operands(g_s, get, 1, h_s)

    def w2_task(c, src):
        tot = [None] * NL
        for r0 in range(0, HN, 16):
            for l, r, y in tiles(src, r0):
                x1 = xn_s[c, l, r:r + 16, :] + y * (0.5 / GS)
                x1_s[c, l, r:r + 16, :] = x1
                tot[l] = x1 if tot[l] is None else tot[l] + x1
            yield 40, [x1_s], (src if r0 + 16 < HN else x1_s)
        yield from ln_stats(tot, lambda l, r: x1_s[c, l, r:r + 16, :], 12, GS, x1_s)
        yield from put_operands(a3, normed(lambda l, r: x1_s[c, l, r:r + 16, :], 12), 2, x1_s)

    def w3_task(src, r0, rn):
        for r in range(0, rn, 16):
            for p, t in enumerate(_act_operands(*[_gelu_scaled(y) for y in quadrants(src, r)])):
                b4[p, (r0 + r) // 2:(r0 + r) // 2 + 8, :] = _pack(t)
            yield 73, [b4], src

    def w4_task(c, src):
        for r0 in range(0, HN, 16):
            for l, r, y in tiles(src, r0):
                y = xb[c, l, r:r + 16, :] + (x1_s[c, l, r:r + 16, :] + y * (0.5 / GS))
                xa[c, l, r:r + 16, :] = y
                ost[c, r:r + 16, l * 128:(l + 1) * 128] = _unpack(_pack(y))
            yield 44, [xa], src

    chunks3, chunks4 = W3_CHUNKS, W4_CHUNKS
    accs, prods = (acc0, acc1), (prod0, prod1, prod2, prod3, prod4)
    group, tune = [0], {}

    def run(name, j, deadline):
        if isinstance(j, int):
            c = j % NS
        elif name == "out":
            c = jnp.where(j[0] < 0, NS, j[0] & (NS - 1))
        else:
            c = j[0] & (NS - 1)
        j = j if isinstance(j, int) else j[1]
        if name == "budget":
            budget[0] = deadline
        elif name[0] == "P":
            spawn((name, 0), deadline, preps[name[1:]][0](), preps[name[1:]][1],
                  after=[t[1] for t in tasks if t[1][0][0] == "P"], delay=ARRIVAL.get(name[1:], 0))
        elif name == "ldx":
            spawn((name, j), deadline, load_x(c), delay=ARRIVAL.get(x_key(c), 0))
        elif name == "ln1":
            spawn((name, j), deadline, ln1_task(c), xa, after=[("ldx", j), ("ln1", j - 1)])
        elif name == "shift":
            spawn((name, j), deadline, shift_task(c), h_s, after=[("w1", j), ("w1", j + 1)])
        elif name == "out":
            acc = accs[(sum(1 for n in chunks4 if n) - 1) % 2]
            finish(("ln4", j))
            spawn((name, j), deadline, w4_task(c, acc), acc, delay=tune["delay"] if slot[0] else 0)
        elif name == "send":
            finish(("out", j))
            for n in range(len(sent), c + 1):
                sent.append(n)
                out_copy(n).start()
        elif name == "ln4":
            spawn((name, j), deadline, w2_task(c, prod_w2), prod_w2, delay=tune["delay"] if slot[0] else 0)
        elif name == "probs":
            spawn((name, j), deadline, probs_task(c), k_s, after=[("q", j), ("k", j), ("attn", j - 1)])
        elif name == "attn":
            spawn((name, j), deadline, attn_out_task(c), v_s, after=[("v", j), ("probs", j)])
        elif name == "w2":
            finish(("shift", j), ("ln4", j - 1), ("Pw2", 0), ("wo", j))
            strassen(w2_s, 0, HN, g_s, prod_w2)
        elif name[:2] == "w4":
            i = int(name[2:])
            r0, rn = sum(chunks4[:i]), chunks4[i]
            if not rn:
                return
            i = sum(1 for n in chunks4[:i] if n)
            finish(("out", j - 1), ("Pw4", 0), *[(f"w3{n}", j) for n in range(len(chunks3)) if sum(chunks3[:n]) < r0 + rn])
            z = zero[0]
            for p in range(7):
                m = product([w4_s[p, kt] for kt in range(r0 // 128, (r0 + rn) // 128)], b4[p, r0 // 2:(r0 + rn) // 2, :])
                accs[i % 2][z, p, 0:HN, :] = accs[(i - 1) % 2][z, p, 0:HN, :] + m if i else m
        else:
            out = prods[group[0] % tune["nbuf"]]
            group[0] += 1
            finish(users.get(id(out)))
            users[id(out)] = (name, j)
            if name[:2] == "w3":
                i = int(name[2:])
                r0, rn = sum(chunks3[:i]), chunks3[i]
                finish(("ln4", j), ("Pw3", 0))
                strassen(w3_s, r0, rn, a3, out)
                gen = w3_task(out, r0, rn)
            else:
                w_ref, r0, b_ref, needs, gen = dict(
                    q=(wqkv_s, 0, a1.at[c & 3], "ln1", q_task(c, out)),
                    k=(wqkv_s, HN, a1.at[c & 3], "ln1", kv_task(c, out, k_s)),
                    v=(wqkv_s, 2 * HN, a1.at[c & 3], "ln1", kv_task(c, out, v_s)),
                    wo=(wo_s, 0, o_s, "attn", wo_task(c, out)),
                    w1=(w1_s, 0, a2, "wo", w1_task(c, out)))[name]
                finish((needs, j), ("P" + name, 0))
                strassen(w_ref, r0, HN, b_ref, out)
            spawn((name, j), deadline, gen, out, delay=tune["delay"])

    def program(params, steps):
        tune.update(params)
        group[0] = slot[0] = credit[0] = 0
        zero[0] = zero_s[0]
        for name, j, deadline in steps:
            run(name, j, deadline)
        finish()
        users.clear()

    users = {}

    for key in ("x0", "q", "k"):
        start(key)
    zero_s[0] = 0
    k_s[0] = jnp.zeros(k_s.shape[1:], u32)
    v_s[0] = jnp.zeros(v_s.shape[1:], u32)
    h_s[0] = jnp.zeros(h_s.shape[1:], f32)
    h_s[NS * NL + 1] = jnp.zeros(h_s.shape[1:], f32)
    for buf in (*[a1.at[n] for n in range(4)], o_s, a2, g_s, a3):
        for p in (3, 4, 6):
            buf[p, K2 // 2:K1 // 2, :] = jnp.zeros(((K1 - K2) // 2, 128), u32)

    def loop(lo, hi, params, steps):
        def body(i, carry):
            program(params, [(name, (i - lag, -lag), deadline) for name, lag, deadline in steps])
            return carry
        lax.fori_loop(lo, hi, body, 0)

    program(*FILL)
    loop(3, NS, *EARLY)

    @pl.when(zero_s[0] > 0)
    def _():
        t, a = of_s[0, 0:256, :], of_s[1, 0:1, :]
        for _ in range(375):
            t = t * a + a
        of_s[0, 0:256, :] = t

    loop(NS, 2 * NS, *STEADY)
    program(*DRAIN)
    for c in range(NS):
        out_copy(c).wait()


@jax.jit
def pallas_interleave_layers__sliding_local_dilated__mixer_s_mlp__prompt_kernel(
    A_x, A_wqkv, A_wo, B_x, B_w1, B_w2, B_w3, B_w4,
):
    del B_x
    nt = NS * NL
    act = pltpu.VMEM((7, K1 // 2, 128), u32)
    res = pltpu.VMEM((NS + 1, NL, D + 8, 128), f32)
    out = pl.pallas_call(
        _kernel,
        out_shape=jax.ShapeDtypeStruct((D, S), bf16),
        in_specs=[pl.BlockSpec(memory_space=pl.ANY)] * 7,
        out_specs=pl.BlockSpec(memory_space=pl.ANY),
        scratch_shapes=[
            pltpu.VMEM((D, S), bf16),
            pltpu.VMEM((D + 16, 3 * D), bf16),
            pltpu.VMEM((D + 16, D), bf16),
            pltpu.VMEM((D + 16, D), bf16),
            pltpu.VMEM((D + 16, D), bf16),
            pltpu.VMEM((D + 16, F), bf16),
            pltpu.VMEM((D + 16, F), bf16),
            pltpu.VMEM((4, F // 2 + 8, 128), u32), pltpu.VMEM((4, HN + 24, 128), u32),
            pltpu.VMEM((7, 2, 3 * HN // 2, 128), u32),
            pltpu.VMEM((7, 2, HN // 2, 128), u32),
            pltpu.VMEM((7, 2, HN // 2, 128), u32),
            pltpu.VMEM((7, 2, HN // 2, 128), u32),
            pltpu.VMEM((7, 2, F // 4, 128), u32),
            pltpu.VMEM((7, F // 256, HN // 2, 128), u32),
            res, res, res, res,
            pltpu.VMEM((nt + 2, D + 8, 128), f32),
            pltpu.VMEM((nt, D, 128), f32),
            pltpu.VMEM((nt + 1, D // 2 + 8, 128), u32),
            pltpu.VMEM((nt + 1, D // 2 + 8, 128), u32),
            pltpu.VMEM((NL, W, H, 128), f32),
            pltpu.VMEM((NL, D + 8, 128), f32),
            pltpu.VMEM((16, 8, 128), f32),
            pltpu.VMEM((4, 7, K1 // 2, 128), u32), act, act, act, act,
            pltpu.VMEM((7, F // 4, 128), u32),
            pltpu.VMEM((1, 7, HN + 8, 128), f32), pltpu.VMEM((1, 7, HN + 8, 128), f32),
            *[pltpu.VMEM((1, 7, 256 + 8, 128), f32)] * (NBUF + 1),
            pltpu.VMEM((1, 8, 128), f32),
            pltpu.VMEM((NS + 1, D, TS), bf16),
            pltpu.SMEM((1,), jnp.int32),
            pltpu.SemaphoreType.DMA((len(X_SPANS),)),
            pltpu.SemaphoreType.DMA((8,)),
            pltpu.SemaphoreType.DMA((NS,)),
        ],
        compiler_params=pltpu.CompilerParams(vmem_limit_bytes=110 * 1024 * 1024),
    )(A_x[0].T, A_wqkv, A_wo, B_w1, B_w2, B_w3, B_w4.T)
    return out.T[None]
```
